```python
import jax
import jax.numpy as jnp

def _softmax(x, axis=-1):
    return jax.nn.softmax(x, axis=axis)
def _gelu(x):
    return jax.nn.gelu(x, approximate=True)
def _silu(x):
    return jax.nn.silu(x)
def _sigmoid(x):
    return jax.nn.sigmoid(x)
def _layernorm(x, axis=-1, eps=1e-5):
    m = jnp.mean(x, axis=axis, keepdims=True)
    v = jnp.var(x, axis=axis, keepdims=True)
    return (x - m) / jnp.sqrt(v + eps)
def _scatter_add(tgt, idx, src, axis=0):
    return tgt.at[idx].add(src)
def _segment_sum(src, seg, n):
    return jax.ops.segment_sum(src, seg, n)
class _Rng:
    def __init__(self, key):
        self._k = key
    def _next(self):
        self._k, sub = jax.random.split(self._k)
        return sub
    def normal(self, shape):
        return jax.random.normal(self._next(), shape, dtype=jnp.bfloat16)
    def randint(self, lo, hi, shape):
        return jax.random.randint(self._next(), shape, lo, hi, dtype=jnp.int32)
    def uniform(self, shape, lo=0.0, hi=1.0):
        return jax.random.uniform(self._next(), shape, jnp.bfloat16, lo, hi)
    def permutation(self, n):
        return jax.random.permutation(self._next(), n)


kernel_name = 'standalone__structured_sparse_n_m__ragged'

def setup_inputs():
    _rng = _Rng(jax.random.key(int.from_bytes(__import__("os").urandom(4), "little")))
    _w = (lambda a: (lambda t: t.astype(jnp.bfloat16) if jnp.issubdtype(t.dtype, jnp.floating) else t)(jnp.asarray(a)))
    B, S, D = 16, 4096, 576
    assert D % 4 == 0, "d_model must be divisible by M=4 for 2:4 sparsity"
    return {
        "x": _w((lambda *s: _rng.normal(s) * 0.05)(B, S, D)),
        "w": _w((lambda *s: _rng.normal(s) * 0.05)(D, D)),
        "b": _w((lambda *s: _rng.normal(s) * 0.05)(D)),
    }

def reference(x, w, b):
    B, S, D = x.shape
    N, M = 2, 4
    G = D // M
    wg = w.reshape(G, M, D)
    mag = jnp.abs(wg)
    order = jnp.argsort(mag, 1)
    thr = jnp.take_along_axis(mag, order[:, M - N:M - N + 1, :], 1)
    mask = (lambda x, dt: x.astype(dt))(mag >= thr, w.dtype)
    wp = (wg * mask).reshape(D, D)
    return jnp.einsum("bsd,df->bsf", x, wp) + b
```

```python
import functools

import jax
import jax.numpy as jnp
import jax.experimental.pallas as pl
import jax.experimental.pallas.tpu as pltpu

GROUP = 4
KEEP = 2
F32 = jnp.float32
BF16 = jnp.bfloat16
H = 288


def _prune(w):
    k = w.shape[0]
    mag = jnp.abs(w)
    pos = jax.lax.broadcasted_iota(jnp.int32, w.shape, 0) % GROUP
    cnt = jnp.zeros(w.shape, jnp.int32)
    for d in range(1, GROUP):
        fwd = pltpu.roll(mag, k - d, 0)
        bwd = pltpu.roll(mag, GROUP - d, 0)
        other = jnp.where(pos + d < GROUP, fwd, bwd)
        cnt = cnt + (other > mag).astype(jnp.int32)
    return jnp.where(cnt < KEEP, w, 0.0)


def _prep(w_ref, b_ref, a_ref, bias_ref):
    wp = _prune(w_ref[...].astype(F32))
    r = jnp.concatenate(
        [wp[0:192], wp[384:448], wp[192:384], wp[448:512], wp[512:576], wp[512:576]], axis=0)
    p = r.T
    pa1, pa2 = p[:H, 0:256], p[H:, 0:256]
    pb1, pb2 = p[:H, 256:512], p[H:, 256:512]
    d1, d2 = p[:H, 512:640], p[H:, 512:640]
    lane = jax.lax.broadcasted_iota(jnp.int32, (H, 256), 1)
    isx = lane < 192
    lane1 = jax.lax.broadcasted_iota(jnp.int32, (H, 128), 1)
    lo = lane1 < 64
    sab = pa1 + pb2
    sa_a = jnp.where(isx, sab, 0.0)
    sa_b = jnp.where(lo, 0.0, sab[:, 128:256])
    sc = pa2 + pb2
    sa_c = jnp.where(isx, sc, -sc)
    sf = pa1 + pb1
    sa_f = jnp.where(isx, sf, -sf)
    sa_d = jnp.where(isx, pa1, pb2)
    sa_e = jnp.where(isx, pb2, pa1)
    s6 = pa2 - pa1
    s7 = pb1 - pb2
    sa_22 = jnp.concatenate([s6[:, :128], jnp.where(lo, s6[:, 128:], d2)], axis=1)
    sa_11 = jnp.concatenate([s7[:, :128], jnp.where(lo, s7[:, 128:], d1)], axis=1)
    sa_21 = jnp.where(lo, d2, s6[:, 128:])
    sa_12 = jnp.where(lo, d1, s7[:, 128:])
    allm = jnp.concatenate([sa_a, sa_b, sa_c, sa_d, sa_e, sa_f, sa_22, sa_11, sa_21, sa_12], axis=1)
    a_ref[...] = pltpu.bitcast(allm.astype(BF16), jnp.uint32)
    bias_ref[...] = jnp.broadcast_to(b_ref[...].astype(F32), (128, b_ref.shape[1])).T


OFF = dict(a=(0, 256), b=(256, 384), c=(384, 640), d=(640, 896), e=(896, 1152), f=(1152, 1408),
           g22=(1408, 1664), g11=(1664, 1920), g21=(1920, 2048), g12=(2048, 2176))


def _pair(x_ref, o_ref, a_ref, bias_ref, c1, c2, w):
    def A(name):
        lo, hi = OFF[name]
        return pltpu.bitcast(a_ref[:, lo:hi], BF16)

    def X(r0, r1, c):
        return x_ref[r0:r1, c:c + w]

    dot = functools.partial(jnp.dot, preferred_element_type=F32)
    cat = lambda *v: jnp.concatenate(v, axis=0)
    xb11, xb12, xb21, xb22 = X(0, 192, c1), X(0, 192, c2), X(192, 384, c1), X(192, 384, c2)
    yb11, yb12, yb21, yb22 = X(384, 448, c1), X(384, 448, c2), X(448, 512, c1), X(448, 512, c2)
    e1, e2 = X(512, 576, c1), X(512, 576, c2)
    f = lambda v: v.astype(F32)
    add = lambda u, v: (f(u) + f(v)).astype(BF16)
    sub = lambda u, v: (f(u) - f(v)).astype(BF16)

    tab = cat(add(xb11, xb22), add(yb12, yb21))
    g_a = dot(A('a'), tab)
    g_b = dot(A('b'), tab[128:256])
    g_c = dot(A('c'), cat(xb11, yb12))
    g_d = dot(A('d'), cat(sub(xb12, xb22), sub(yb22, yb12)))
    g_e = dot(A('e'), cat(sub(xb21, xb11), sub(yb11, yb21)))
    g_f = dot(A('f'), cat(xb22, yb21))
    g_22 = dot(A('g22'), cat(add(xb11, xb12), e2))
    g_11 = dot(A('g11'), cat(add(xb21, xb22), e1))
    g_21 = dot(A('g21'), cat(e1, add(yb12, yb11)))
    g_12 = dot(A('g12'), cat(e2, add(yb22, yb21)))
    rep = lambda v: jnp.concatenate([v] * (w // 128), axis=1) if w > 128 else v
    b1, b2 = rep(bias_ref[:H]), rep(bias_ref[H:])
    o_ref[:H, c1:c1 + w] = (g_a + g_e - g_f + g_11 + b1).astype(BF16)
    o_ref[H:, c2:c2 + w] = (g_a - g_c + g_d + g_22 + b2).astype(BF16)
    o_ref[:H, c2:c2 + w] = (g_b + g_d + g_f + g_12 + b1).astype(BF16)
    o_ref[H:, c1:c1 + w] = (g_b + g_c + g_e + g_21 + b2).astype(BF16)


def _kernel(x_hbm, w_hbm, b_hbm, o_hbm, xbuf, obuf, wbuf, bbuf, a_ref, bias_ref, rsem, wsem, hsem, tsem, msem,
            *, pw, head, tail, nout, wstart, inl):
    B, D, S = x_hbm.shape

    wcp = pltpu.make_async_copy(w_hbm, wbuf, msem.at[0])
    bcp = pltpu.make_async_copy(b_hbm, bbuf, msem.at[1])
    wcp.start()
    bcp.start()

    def cuts(sizes):
        o, r = 0, []
        for s in sizes:
            r.append((o, s)); o += s
        assert o == S
        return r

    hc, tc = cuts(head), cuts(tail)
    def rd_head(u):
        o, s = hc[u]
        return pltpu.make_async_copy(x_hbm.at[0, :, pl.ds(o, s)], xbuf.at[0, :, pl.ds(o, s)], hsem.at[u])
    def rd(i):
        return pltpu.make_async_copy(x_hbm.at[i], xbuf.at[i], rsem.at[i])
    def wr(i):
        return pltpu.make_async_copy(obuf.at[i % nout], o_hbm.at[i], wsem.at[i])
    def wr_tail(u):
        o, s = tc[u]
        return pltpu.make_async_copy(obuf.at[(B - 1) % nout, :, pl.ds(o, s)], o_hbm.at[B - 1, :, pl.ds(o, s)], tsem.at[u])

    for u in range(len(hc)):
        rd_head(u).start()
    for i in range(1, B):
        rd(i).start()

    wcp.wait()
    bcp.wait()
    _prep(wbuf, bbuf, a_ref, bias_ref)

    def compute(i, o, s):
        xr, orf = xbuf.at[i], obuf.at[i % nout]
        for p in range(s // (2 * pw)):
            _pair(xr, orf, a_ref, bias_ref, o + p * 2 * pw, o + p * 2 * pw + pw, pw)

    for u, (o, s) in enumerate(hc):
        rd_head(u).wait()
        compute(0, o, s)

    def body(i, _):
        rd(i).wait()

        @pl.when(i >= nout)
        def _():
            wr(i - nout).wait()

        @pl.when(i == wstart)
        def _():
            for j in range(wstart):
                wr(j).start()

        @pl.when(i > wstart)
        def _():
            wr(i - 1).start()

        compute(i, 0, S)
        return 0

    jax.lax.fori_loop(1, B - 1, body, 0)

    rd(B - 1).wait()
    wr(B - 1 - nout).wait()
    wr(B - 2).start()
    for u, (o, s) in enumerate(tc):
        compute(B - 1, o, s)
        wr_tail(u).start()
    for j in range(B - nout, B - 1):
        wr(j).wait()
    for u in range(len(tc)):
        wr_tail(u).wait()


@functools.partial(jax.jit, static_argnames=("pw", "head", "tail", "nout", "wstart", "inl"))
def pallas_standalone__structured_sparse_n_m__ragged_kernel(
        x, w, b, pw=128, head=(1024, 1024, 2048), tail=(2048, 1536, 512), nout=9, wstart=7, inl=0):
    B, S, D = x.shape
    xt = jnp.transpose(x, (0, 2, 1))
    out_t = pl.pallas_call(
        functools.partial(_kernel, pw=pw, head=head, tail=tail, nout=nout, wstart=wstart, inl=inl),
        in_specs=[pl.BlockSpec(memory_space=pl.ANY)] * 3,
        out_specs=pl.BlockSpec(memory_space=pl.ANY),
        out_shape=jax.ShapeDtypeStruct((B, D, S), x.dtype),
        scratch_shapes=[
            pltpu.VMEM((B, D, S), BF16),
            pltpu.VMEM((nout, D, S), BF16),
            pltpu.VMEM((D, D), BF16),
            pltpu.VMEM((1, D), BF16),
            pltpu.VMEM((144, 2176), jnp.uint32),
            pltpu.VMEM((D, 128), F32),
            pltpu.SemaphoreType.DMA((B,)),
            pltpu.SemaphoreType.DMA((B,)),
            pltpu.SemaphoreType.DMA((len(head),)),
            pltpu.SemaphoreType.DMA((len(tail),)),
            pltpu.SemaphoreType.DMA((2,)),
        ],
        compiler_params=pltpu.CompilerParams(
            vmem_limit_bytes=126 * 1024 * 1024,
        ),
    )(xt, w, b.reshape(1, D))
    return jnp.transpose(out_t, (0, 2, 1))
```

```python
import functools

import jax
import jax.numpy as jnp
import jax.experimental.pallas as pl
import jax.experimental.pallas.tpu as pltpu

F32, BF16, U32, I32 = jnp.float32, jnp.bfloat16, jnp.uint32, jnp.int32
H = 288
Q = 144
QW = 512
W1 = 256
W2 = 128
GROUPS = ('a', 'b', 'c', 'd', 'e', 'f', 'g22', 'g11', 'g21', 'g12')
KW = dict(a=256, b=128, c=256, d=256, e=256, f=256, g22=256, g11=256, g21=128, g12=128)
USES = dict(a=((11, 1), (22, -1)), b=((12, -1), (21, 1)), c=((21, 1), (22, 1)), d=((12, 1), (22, 1)),
            e=((11, 1), (21, 1)), f=((11, 1), (12, 1)), g11=((11, 1),), g22=((22, 1),), g12=((12, 1),),
            g21=((21, 1),))


def _layout(l2):
    o1, o2, off = 0, 0, {}
    for g in GROUPS:
        if g in l2:
            off[g] = o2; o2 += 7 * 128
        else:
            off[g] = o1; o1 += KW[g]
    return off, o1, max(o2, 128)


def _swap_pairs(v):
    n, L = v.shape
    v3 = v.reshape(n // 8, 8, L)
    up = pltpu.roll(v3, 7, 1)
    dn = pltpu.roll(v3, 1, 1)
    odd = (jax.lax.broadcasted_iota(I32, v3.shape, 1) & 1) == 1
    return jnp.where(odd, dn, up).reshape(n, L)


def _prune(wb):
    u = pltpu.bitcast(wb, U32)
    f = lambda v: pltpu.bitcast(v, F32)
    lo = f((u << 16) & jnp.uint32(0x7FFF0000))
    hi = f(u & jnp.uint32(0x7FFF0000))
    a, b = jnp.maximum(lo, hi), jnp.minimum(lo, hi)
    a2, b2 = _swap_pairs(a), _swap_pairs(b)
    thr = jnp.maximum(jnp.minimum(a, a2), jnp.maximum(b, b2))
    keep = (jnp.where(lo >= thr, jnp.uint32(0x0000FFFF), jnp.uint32(0))
            | jnp.where(hi >= thr, jnp.uint32(0xFFFF0000), jnp.uint32(0)))
    return pltpu.bitcast(u & keep, BF16)


def _prep(w_ref, b_ref, a1_ref, a2_ref, bias_ref, l2):
    wp = _prune(w_ref[...])
    r = jnp.concatenate([wp[0:192], wp[384:448], wp[192:384], wp[448:512], wp[512:576], wp[512:576]], axis=0)
    p = r.T.astype(F32)
    pa1, pa2 = p[:H, 0:256], p[H:, 0:256]
    pb1, pb2 = p[:H, 256:512], p[H:, 256:512]
    d1, d2 = p[:H, 512:640], p[H:, 512:640]
    lo = jax.lax.broadcasted_iota(I32, (H, 128), 1) < 64
    mix = lambda u, v: jnp.concatenate([u[:, :128], jnp.where(lo, u[:, 128:], v[:, -128:])], axis=1)
    sab = pa1 + pb2
    s6 = pa2 - pa1
    s7 = pb1 - pb2
    zero = jnp.zeros((H, 128), F32)
    sa = dict(
        a=mix(sab, zero),
        b=jnp.where(lo, zero, sab[:, 128:]),
        c=pa2 + pb2,
        f=pa1 + pb1,
        d=mix(pa1, pb2),
        e=mix(pb2, pa1),
        g22=mix(s6, d2),
        g11=mix(s7, d1),
        g21=jnp.where(lo, d2, s6[:, 128:]),
        g12=jnp.where(lo, d1, s7[:, 128:]),
    )
    off, _, _ = _layout(l2)
    for g in GROUPS:
        m = sa[g]
        if g in l2:
            p11, p12, p21, p22 = m[:Q, :128], m[:Q, 128:], m[Q:, :128], m[Q:, 128:]
            m = jnp.concatenate([p11 + p22, p21 + p22, p11, p22, p11 + p12, p21 - p11, p12 - p22], axis=1)
            a2_ref[:, off[g]:off[g] + 896] = pltpu.bitcast(m.astype(BF16), U32)
        else:
            a1_ref[:, off[g]:off[g] + KW[g]] = pltpu.bitcast(m.astype(BF16), U32)
    bv = b_ref[...].astype(F32).reshape(1, 2 * H)
    bias_ref[...] = jnp.broadcast_to(bv, (128, 2 * H)).T


def _quad(x_ref, o_ref, a1_ref, a2_ref, bias_ref, fence_ref, c1, l2, order, opt, after_store=None):
    c2 = c1 + W1
    off, _, _ = _layout(l2)
    dot = functools.partial(jnp.dot, preferred_element_type=F32)
    cat = lambda v: jnp.concatenate(v, axis=0) if len(v) > 1 else v[0]

    def fence():
        fence_ref[0] = jnp.int32(0)

    def pieces(op, r0, r1):
        base = 0
        for n, terms in op:
            lo, hi = max(r0, base), min(r1, base + n)
            if lo < hi:
                yield lo, hi, [(sg, rr + lo - base, cc) for sg, rr, cc in terms]
            base += n

    def seg(terms, n, col, ww):
        pos = [t for t in terms if t[0] > 0] + [t for t in terms if t[0] < 0]
        acc = None
        for sg, rr, cc in pos:
            v = x_ref[rr:rr + n, cc + col:cc + col + ww].astype(F32)
            acc = (v if sg > 0 else -v) if acc is None else (acc + v if sg > 0 else acc - v)
        return acc

    def tile(op, combo, k, ww, trim=False):
        cuts = sorted({0, k} | {lo - r0 for _, r0, _ in combo for lo, _, _ in pieces(op, r0, r0 + k)})
        parts, allraw = [], True
        for lo, hi in zip(cuts[:-1], cuts[1:]):
            per = []
            for sg, r0, col in combo:
                (_, _, terms), = pieces(op, r0 + lo, r0 + hi)
                if terms:
                    per.append((sg, terms, col))
            nterms = sum(len(t) for _, t, _ in per)
            raw = nterms == 1 and per[0][0] * per[0][1][0][0] > 0
            allraw = allraw and (raw or nterms == 0)
            parts.append((lo, hi, per, raw))
        if trim:
            while parts and not parts[-1][2]:
                parts.pop()
        out = []
        for lo, hi, per, raw in parts:
            n = hi - lo
            if not per:
                out.append(jnp.zeros((n, ww), BF16 if allraw else F32))
            elif allraw:
                _, ((_, rr, cc),), col = per[0]
                out.append(x_ref[rr:rr + n, cc + col:cc + col + ww])
            else:
                per = [p for p in per if p[0] > 0] + [p for p in per if p[0] < 0]
                acc = None
                for sg, terms, col in per:
                    v = seg(terms, n, col, ww)
                    acc = (v if sg > 0 else -v) if acc is None else (acc + v if sg > 0 else acc - v)
                out.append(acc)
        return cat(out).astype(BF16)

    def prod(g, op, bias):
        fence()
        if g not in l2:
            t = tile(op, [(1, 0, 0)], KW[g], W1, trim=True)
            a = pltpu.bitcast(a1_ref[:, off[g]:off[g] + KW[g]], BF16)
            r = dot(a[:, :t.shape[0]], t)
            return r if bias is None else r + jnp.concatenate([bias, bias], axis=1)
        combos = [[(1, 0, 0), (1, 128, W2)], [(1, 0, 0)], [(1, 0, W2), (-1, 128, W2)], [(1, 128, 0), (-1, 0, 0)],
                  [(1, 128, W2)], [(1, 0, 0), (1, 0, W2)], [(1, 128, 0), (1, 128, W2)]]
        m = {}
        for i in opt.get('mo', (0, 3, 4, 6, 1, 2, 5)):
            t = tile(op, combos[i], 128, W2, trim=True)
            a = pltpu.bitcast(a2_ref[:, off[g] + 128 * i:off[g] + 128 * (i + 1)], BF16)
            m[i + 1] = dot(a[:, :t.shape[0]], t)
        g11, g12, g21, g22 = m[1] + m[4] - m[5] + m[7], m[5] + m[3], m[4] + m[2], m[1] - m[2] + m[3] + m[6]
        if bias is not None:
            g11, g12, g21, g22 = g11 + bias[:Q], g12 + bias[:Q], g21 + bias[Q:], g22 + bias[Q:]
        return jnp.concatenate([jnp.concatenate([g11, g12], axis=1), jnp.concatenate([g21, g22], axis=1)], axis=0)

    x11, x12, x21, x22 = (0, c1), (0, c2), (192, c1), (192, c2)
    y11, y12, y21, y22 = (384, c1), (384, c2), (448, c1), (448, c2)
    e1, e2 = (512, c1), (512, c2)
    P = lambda u: (1,) + u
    M = lambda u: (-1,) + u
    ops = dict(
        a=[(192, [P(x11), M(x22)]), (64, [])],
        b=[(64, []), (64, [P(y21), M(y12)])],
        c=[(192, [P(x11)]), (64, [P(y12)])],
        d=[(192, [P(x12), M(x22)]), (64, [P(y22), M(y12)])],
        e=[(192, [P(x21), M(x11)]), (64, [P(y11), M(y21)])],
        f=[(192, [P(x22)]), (64, [P(y21)])],
        g22=[(192, [P(x12), M(x11)]), (64, [P(e2)])],
        g11=[(192, [P(x21), M(x22)]), (64, [P(e1)])],
        g21=[(64, [P(e1)]), (64, [P(y11), M(y12)])],
        g12=[(64, [P(e2)]), (64, [P(y22), M(y21)])],
    )
    where = {11: (0, c1), 12: (0, c2), 21: (H, c1), 22: (H, c2)}
    left = {k: 4 for k in where}
    acc, neg = {}, {}
    for g in order:
        bias = {'f': lambda: bias_ref[:H], 'c': lambda: bias_ref[H:]}.get(g, lambda: None)()
        v = prod(g, ops[g], bias)
        for k, sg in USES[g]:
            if k not in acc:
                acc[k], neg[k] = v, sg < 0
            elif neg[k]:
                assert sg > 0
                acc[k], neg[k] = v - acc[k], False
            else:
                acc[k] = acc[k] + v if sg > 0 else acc[k] - v
            left[k] -= 1
            if left[k] == 0:
                r0, cc = where[k]
                o_ref[r0:r0 + H, cc:cc + W1] = acc[k].astype(BF16)
                if after_store is not None:
                    after_store(r0, cc)


def _kernel(x_hbm, w_hbm, b_hbm, o_hbm, xbuf, obuf, wbuf, bbuf, a1_ref, a2_ref, bias_ref, fence_ref,
            rsem, wsem, hsem, msem, *, l2, order, opt, nout, t0, mode, lastp, selft, nkick, small_tail):
    B, D, S = x_hbm.shape
    NB, R = D // 64, 64
    WC = 1024
    nq, nj, nr = S // QW, S // WC, R // 8
    nqh = 2
    npc, pw = nq // nqh, nqh * QW
    obuf_v = obuf.reshape(nout * NB, R, S)
    quad = functools.partial(_quad, a1_ref=a1_ref, a2_ref=a2_ref, bias_ref=bias_ref, fence_ref=fence_ref,
                             l2=l2, order=order, opt=opt)
    RD, WR = 'r' in mode, 'w' in mode

    wcp = pltpu.make_async_copy(w_hbm, wbuf, msem.at[0])
    bcp = pltpu.make_async_copy(b_hbm, bbuf, msem.at[1])
    wcp.start()
    bcp.start()

    def rd_head(u):
        col = pl.multiple_of(u * pw, pw)
        return pltpu.make_async_copy(x_hbm.at[0, :, pl.ds(col, pw)], xbuf.at[0, :, pl.ds(col, pw)], hsem.at[u])

    def rd(i):
        return pltpu.make_async_copy(x_hbm.at[i], xbuf.at[i], rsem.at[i])

    def rd_last(u):
        r0, n = (0, D - lastp) if u == 0 else (D - lastp, lastp)
        return pltpu.make_async_copy(x_hbm.at[B - 1, pl.ds(r0, n)], xbuf.at[B - 1, pl.ds(r0, n)],
                                     rsem.at[B - 1] if u == 0 else rsem.at[0])

    def slot(i):
        return i % nout if isinstance(i, int) else jnp.where(i >= nout, i - nout, i)

    def wr_chunk(i, nb, r, j, sem):
        col = j * WC if isinstance(j, int) else pl.multiple_of(j * WC, WC)
        return pltpu.make_async_copy(obuf_v.at[pl.ds(slot(i) * NB, nb * NB), pl.ds(r * 8, 8), pl.ds(col, WC)],
                                     o_hbm.at[pl.ds(i * NB, nb * NB), pl.ds(r * 8, 8), pl.ds(col, WC)], sem)

    def wr_wait(i, nb, sem):
        pltpu.make_async_copy(obuf_v.at[pl.ds(slot(i) * NB, nb * NB)], o_hbm.at[pl.ds(i * NB, nb * NB)], sem).wait()

    def loop(lo, hi, f):
        def body(i, c):
            f(i)
            return c
        jax.lax.fori_loop(lo, hi, body, 0)

    if RD:
        loop(0, npc, lambda u: rd_head(u).start())
        loop(1, B - 1, lambda i: rd(i).start())
        loop(0, 1, lambda _: rd_last(0).start())
        if lastp:
            loop(0, 1, lambda _: rd_last(1).start())

    wcp.wait()
    bcp.wait()
    _prep(wbuf, bbuf, a1_ref, a2_ref, bias_ref, l2)

    def head_step(u):
        if RD:
            rd_head(u).wait()
        col = pl.multiple_of(u * pw, pw)
        xr, orf = xbuf.at[0, :, pl.ds(col, pw)], obuf.at[0, :, pl.ds(col, pw)]
        for k in range(nqh):
            quad(xr, orf, c1=k * QW)

    loop(0, npc, head_step)

    npair = (B - 2) // 2
    assert nout % 2 == 0 and t0 + npair == B - 1 and 2 * (npair - 1) + 1 < t0 + npair - 1
    for i in range(nout, B):
        assert t0 + (i - nout) // 2 < i

    def mid_step(i):
        if RD:
            rd(i).wait()
        if WR:
            reuse = jnp.logical_and(i >= nout, jax.lax.bitwise_and(i, 1) == 0)
            loop(0, reuse.astype(I32), lambda _: wr_wait(i - nout, 2, wsem.at[jax.lax.shift_right_logical(i - nout, 1)]))
            p = jnp.maximum(i - t0, 0)
            first = (i == t0).astype(I32)
            if RD and selft:
                loop(0, first, lambda _: rd_last(0).wait())

            def kick(_):
                for u in range(nkick):
                    wr_chunk(0, 2, u // nj, u % nj, wsem.at[0]).start()
            if nkick:
                loop(0, first, kick)
            for r in range(nr):
                for j in range(nj):
                    @pl.when(i >= t0 + (1 if r * nj + j < nkick else 0))
                    def _():
                        wr_chunk(2 * p, 2, r, j, wsem.at[p]).start()
        for k in range(nq):
            quad(xbuf.at[i], obuf.at[slot(i)], c1=k * QW)

    loop(1, B - 1, mid_step)

    last = B - 1
    if RD:
        if not (selft and WR):
            rd_last(0).wait()
        if lastp:
            rd_last(1).wait()
    waited = {(i - nout) // 2 for i in range(nout, B - 1) if i % 2 == 0}
    assert (last - nout) // 2 in waited
    if small_tail:
        def tail_step(u):
            if WR:
                for r in range(nr):
                    for j in range(nj):
                        @pl.when(u == 0)
                        def _():
                            wr_chunk(last - 1, 1, r, j, wsem.at[npair]).start()
                for r in range(nr):
                    @pl.when(u > 0)
                    def _():
                        wr_chunk(last, 1, r, jnp.maximum(u - 1, 0), wsem.at[npair + 1]).start()
            col = pl.multiple_of(u * pw, pw)
            xr, orf = xbuf.at[last, :, pl.ds(col, pw)], obuf.at[slot(last), :, pl.ds(col, pw)]
            for k in range(nqh):
                quad(xr, orf, c1=k * QW)

        loop(0, npc, tail_step)
        if WR:
            for r in range(nr):
                wr_chunk(last, 1, r, nj - 1, wsem.at[npair + 1]).start()
    else:
        if WR:
            for r in range(nr):
                for j in range(nj):
                    wr_chunk(last - 1, 1, r, j, wsem.at[npair]).start()
        for k in range(nq):
            fine = WR and k >= nq - 2

            def after(r0, cc):
                pltpu.make_async_copy(obuf.at[slot(last), pl.ds(r0, H), pl.ds(cc, W1)],
                                      o_hbm.reshape(B, D, S).at[last, pl.ds(r0, H), pl.ds(cc, W1)], wsem.at[npair + 1]).start()

            quad(xbuf.at[last], obuf.at[slot(last)], c1=k * QW, after_store=after if fine else None)
            if WR and not fine and (k + 1) % (WC // QW) == 0:
                for r in range(nr):
                    wr_chunk(last, 1, r, k // (WC // QW), wsem.at[npair + 1]).start()
    if WR:
        for p in range(npair):
            if p not in waited:
                wr_wait(2 * p, 2, wsem.at[p])
        wr_wait(last - 1, 1, wsem.at[npair])
        wr_wait(last, 1, wsem.at[npair + 1])


@functools.partial(jax.jit, static_argnames=("l2", "order", "mo", "nout", "t0", "mode", "lastp", "selft", "nkick", "small_tail"))
def pallas_standalone__structured_sparse_n_m__ragged_kernel(
        x, w, b, l2='a+c+d+e+f+g11+g22', order='a+b+g11+e+g21+f+c+g12+g22+d', mo=(0, 3, 4, 6, 1, 2, 5),
        nout=10, t0=8, mode='rw', lastp=48, selft=1, nkick=8, small_tail=1):
    B, S, D = x.shape
    l2 = tuple(l2.split('+')) if l2 else ()
    _, n1, n2 = _layout(l2)
    xt = jnp.transpose(x, (0, 2, 1))
    out_t = pl.pallas_call(
        functools.partial(_kernel, l2=l2, order=tuple(order.split('+')), opt=dict(mo=mo), nout=nout, t0=t0, mode=mode, lastp=lastp, selft=selft, nkick=nkick, small_tail=small_tail),
        in_specs=[pl.BlockSpec(memory_space=pl.ANY)] * 3,
        out_specs=pl.BlockSpec(memory_space=pl.ANY),
        out_shape=jax.ShapeDtypeStruct((B * D // 64, 64, S), x.dtype),
        scratch_shapes=[
            pltpu.VMEM((B, D, S), BF16),
            pltpu.VMEM((nout, D, S), BF16),
            pltpu.VMEM((D, D), BF16),
            pltpu.VMEM((D,), BF16),
            pltpu.VMEM((144, n1), U32),
            pltpu.VMEM((72, n2), U32),
            pltpu.VMEM((D, 128), F32),
            pltpu.SMEM((1,), I32),
            pltpu.SemaphoreType.DMA((B,)),
            pltpu.SemaphoreType.DMA((B // 2 + 1,)),
            pltpu.SemaphoreType.DMA((S // 1024,)),
            pltpu.SemaphoreType.DMA((2,)),
        ],
        compiler_params=pltpu.CompilerParams(
            vmem_limit_bytes=127 * 1024 * 1024,
            disable_bounds_checks=True,
        ),
    )(xt, w, b)
    return jnp.transpose(out_t.reshape(B, D, S), (0, 2, 1))
```

```python
import functools

import jax
import jax.numpy as jnp
import jax.experimental.pallas as pl
import jax.experimental.pallas.tpu as pltpu

F32, BF16, U32, I32 = jnp.float32, jnp.bfloat16, jnp.uint32, jnp.int32

D = 576
H = D // 2
Q = H // 2
W1 = 256
W2 = 128
QW = 2 * W1

KW = dict(a=256, b=128, c=256, d=256, e=256, f=256, g22=256, g11=256, g21=128, g12=128)
USES = dict(a=((11, 1), (22, -1)), b=((12, -1), (21, 1)), c=((21, 1), (22, 1)), d=((12, 1), (22, 1)),
            e=((11, 1), (21, 1)), f=((11, 1), (12, 1)), g11=((11, 1),), g22=((22, 1),), g12=((12, 1),),
            g21=((21, 1),))
LEVEL2 = ('a', 'c', 'd', 'e', 'f', 'g22', 'g11')
ORDER = ('a', 'b', 'g11', 'e', 'g21', 'f', 'c', 'g12', 'g22', 'd')
A1_OFF = dict(b=0, g21=128, g12=256)
A2_OFF = {g: 7 * 128 * i for i, g in enumerate(LEVEL2)}

NOUT = 10
T0 = 8
LASTP = 48
WC = 1024
NSMALL = 2
NPTS = 4
NKICK = 4


def _swap_pairs(v):
    n, lanes = v.shape
    v3 = v.reshape(n // 8, 8, lanes)
    up = pltpu.roll(v3, 7, 1)
    dn = pltpu.roll(v3, 1, 1)
    odd = (jax.lax.broadcasted_iota(I32, v3.shape, 1) & 1) == 1
    return jnp.where(odd, dn, up).reshape(n, lanes)


def _prune(wb):
    u = pltpu.bitcast(wb, U32)
    lo = pltpu.bitcast((u << 16) & jnp.uint32(0x7FFF0000), F32)
    hi = pltpu.bitcast(u & jnp.uint32(0x7FFF0000), F32)
    big, small = jnp.maximum(lo, hi), jnp.minimum(lo, hi)
    thr = jnp.maximum(jnp.minimum(big, _swap_pairs(big)), jnp.maximum(small, _swap_pairs(small)))
    keep = (jnp.where(lo >= thr, jnp.uint32(0x0000FFFF), jnp.uint32(0))
            | jnp.where(hi >= thr, jnp.uint32(0xFFFF0000), jnp.uint32(0)))
    return pltpu.bitcast(u & keep, BF16)


def _prepare(w_ref, b_ref, a1_ref, a2_ref, bias_ref):
    wp = _prune(w_ref[...])
    r = jnp.concatenate([wp[0:192], wp[384:448], wp[192:384], wp[448:512], wp[512:576], wp[512:576]], axis=0)
    p = r.T.astype(F32)
    a11, a21 = p[:H, 0:256], p[H:, 0:256]
    a12, a22 = p[:H, 256:512], p[H:, 256:512]
    e1, e2 = p[:H, 512:640], p[H:, 512:640]
    low = jax.lax.broadcasted_iota(I32, (H, 128), 1) < 64
    mix = lambda u, v: jnp.concatenate([u[:, :128], jnp.where(low, u[:, 128:], v[:, -128:])], axis=1)
    zero = jnp.zeros((H, 128), F32)
    s1, s6, s7 = a11 + a22, a21 - a11, a12 - a22
    sa = dict(a=mix(s1, zero), b=jnp.where(low, zero, s1[:, 128:]), c=a21 + a22, d=mix(a11, a22), e=mix(a22, a11),
              f=a11 + a12, g22=mix(s6, e2), g11=mix(s7, e1), g21=jnp.where(low, e2, s6[:, 128:]),
              g12=jnp.where(low, e1, s7[:, 128:]))
    for g, m in sa.items():
        if g in LEVEL2:
            p11, p12, p21, p22 = m[:Q, :128], m[:Q, 128:], m[Q:, :128], m[Q:, 128:]
            m = jnp.concatenate([p11 + p22, p21 + p22, p11, p22, p11 + p12, p21 - p11, p12 - p22], axis=1)
            a2_ref[:, A2_OFF[g]:A2_OFF[g] + 7 * 128] = pltpu.bitcast(m.astype(BF16), U32)
        else:
            a1_ref[:, A1_OFF[g]:A1_OFF[g] + KW[g]] = pltpu.bitcast(m.astype(BF16), U32)
    bias_ref[...] = jnp.broadcast_to(b_ref[...].astype(F32).reshape(1, D), (128, D)).T


def _signed_sum(items):
    acc = None
    for sign, get in sorted(items, key=lambda t: -t[0]):
        v = get()
        acc = (v if sign > 0 else -v) if acc is None else (acc + v if sign > 0 else acc - v)
    return acc


def _quad(x_ref, o_ref, a1_ref, a2_ref, bias_ref, fence_ref, c1):
    c2 = c1 + W1
    dot = functools.partial(jnp.dot, preferred_element_type=F32)

    x11, x12, x21, x22 = (0, c1), (0, c2), (192, c1), (192, c2)
    y11, y12, y21, y22 = (384, c1), (384, c2), (448, c1), (448, c2)
    e1, e2 = (512, c1), (512, c2)
    pos, neg = (lambda u: (1,) + u), (lambda u: (-1,) + u)
    operand = dict(
        a=[(192, [pos(x11), neg(x22)]), (64, [])],
        b=[(64, []), (64, [pos(y21), neg(y12)])],
        c=[(192, [pos(x11)]), (64, [pos(y12)])],
        d=[(192, [pos(x12), neg(x22)]), (64, [pos(y22), neg(y12)])],
        e=[(192, [pos(x21), neg(x11)]), (64, [pos(y11), neg(y21)])],
        f=[(192, [pos(x22)]), (64, [pos(y21)])],
        g22=[(192, [pos(x12), neg(x11)]), (64, [pos(e2)])],
        g11=[(192, [pos(x21), neg(x22)]), (64, [pos(e1)])],
        g21=[(64, [pos(e1)]), (64, [pos(y11), neg(y12)])],
        g12=[(64, [pos(e2)]), (64, [pos(y22), neg(y21)])],
    )

    def terms_at(op, row):
        base = 0
        for n, terms in op:
            if base <= row < base + n:
                return [(sg, rr + row - base, cc) for sg, rr, cc in terms]
            base += n

    def tile(op, combo, k, width):
        parts = []
        for lo in range(0, k, 64):
            parts.append([(sg, terms_at(op, r0 + lo), col) for sg, r0, col in combo if terms_at(op, r0 + lo)])
        while not parts[-1]:
            parts.pop()
        load = lambda rr, cc: x_ref[rr:rr + 64, cc:cc + width]
        raw = all(not p or (len(p) == 1 and len(p[0][1]) == 1 and p[0][0] * p[0][1][0][0] > 0) for p in parts)
        out = []
        for p in parts:
            if not p:
                out.append(jnp.zeros((64, width), BF16 if raw else F32))
            elif raw:
                out.append(load(p[0][1][0][1], p[0][1][0][2] + p[0][2]))
            else:
                inner = lambda ts, col: _signed_sum(
                    [(sg, lambda rr=rr, cc=cc: load(rr, cc + col).astype(F32)) for sg, rr, cc in ts])
                out.append(_signed_sum([(sg, lambda ts=ts, col=col: inner(ts, col)) for sg, ts, col in p]))
        return (jnp.concatenate(out, axis=0) if len(out) > 1 else out[0]).astype(BF16)

    def product(g, bias):
        fence_ref[0] = jnp.int32(0)
        op = operand[g]
        if g not in LEVEL2:
            a = pltpu.bitcast(a1_ref[:, A1_OFF[g]:A1_OFF[g] + KW[g]], BF16)
            return dot(a, tile(op, [(1, 0, 0)], KW[g], W1))
        combos = ([(1, 0, 0), (1, 128, W2)], [(1, 0, 0)], [(1, 0, W2), (-1, 128, W2)], [(1, 128, 0), (-1, 0, 0)],
                  [(1, 128, W2)], [(1, 0, 0), (1, 0, W2)], [(1, 128, 0), (1, 128, W2)])
        m = {}
        for i in (0, 3, 4, 6, 1, 2, 5):
            t = tile(op, combos[i], 128, W2)
            a = pltpu.bitcast(a2_ref[:, A2_OFF[g] + 128 * i:A2_OFF[g] + 128 * (i + 1)], BF16)
            m[i + 1] = dot(a[:, :t.shape[0]], t)
        g11, g12, g21, g22 = m[1] + m[4] - m[5] + m[7], m[5] + m[3], m[4] + m[2], m[1] - m[2] + m[3] + m[6]
        if bias is not None:
            g11, g12, g21, g22 = g11 + bias[:Q], g12 + bias[:Q], g21 + bias[Q:], g22 + bias[Q:]
        return jnp.concatenate([jnp.concatenate([g11, g12], axis=1), jnp.concatenate([g21, g22], axis=1)], axis=0)

    corner = {11: (0, c1), 12: (0, c2), 21: (H, c1), 22: (H, c2)}
    left = {k: 4 for k in corner}
    acc, flipped = {}, {}
    for g in ORDER:
        bias = bias_ref[:H] if g == 'f' else bias_ref[H:] if g == 'c' else None
        v = product(g, bias)
        for k, sign in USES[g]:
            if k not in acc:
                acc[k], flipped[k] = v, sign < 0
            elif flipped[k]:
                assert sign > 0
                acc[k], flipped[k] = v - acc[k], False
            else:
                acc[k] = acc[k] + v if sign > 0 else acc[k] - v
            left[k] -= 1
            if left[k] == 0:
                r0, cc = corner[k]
                o_ref[r0:r0 + H, cc:cc + W1] = acc[k].astype(BF16)


def _loop(lo, hi, f):
    def body(i, carry):
        f(i)
        return carry
    jax.lax.fori_loop(lo, hi, body, 0)


def _once_if(cond, f):
    _loop(0, cond.astype(I32), lambda _: f())


def _kernel(x_hbm, w_hbm, b_hbm, o_hbm, xbuf, obuf, wbuf, bbuf, a1_ref, a2_ref, bias_ref, fence_ref,
            rsem, wsem, hsem, msem):
    nbatch, _, seq = x_hbm.shape
    last = nbatch - 1
    nb = D // 64
    nq, nj = seq // QW, seq // WC
    npc, pw = nq // NSMALL, NSMALL * QW
    npair = (nbatch - 2) // 2
    obuf_1, obuf_2 = obuf.reshape(NOUT * nb, 64, seq), obuf.reshape(NOUT * nb // 2, 128, seq)
    out_1, out_2 = o_hbm, o_hbm.reshape(nbatch * nb // 2, 128, seq)
    band, shr = jax.lax.bitwise_and, jax.lax.shift_right_logical
    both, either = jnp.logical_and, jnp.logical_or

    assert pw == WC and NOUT % 2 == 0 and nbatch <= 2 * NOUT
    assert T0 + npair == last and all(2 * p + 1 < T0 + p for p in range(npair))
    assert all(T0 + (i - NOUT) // 2 < i - i % 2 for i in range(NOUT, nbatch))
    waited = {(i - NOUT) // 2 for i in range(NOUT, last) if i % 2 == 0}
    assert (last - NOUT) // 2 in waited

    def slab(i):
        return i % NOUT if isinstance(i, int) else jnp.where(i >= NOUT, i - NOUT, i)

    def rd_head(u):
        col = pl.multiple_of(u * pw, pw)
        return pltpu.make_async_copy(x_hbm.at[0, :, pl.ds(col, pw)], xbuf.at[0, :, pl.ds(col, pw)], hsem.at[u])

    def rd(i):
        return pltpu.make_async_copy(x_hbm.at[i], xbuf.at[i], rsem.at[i])

    def rd_last(part):
        rows = pl.ds(0, D - LASTP) if part == 0 else pl.ds(D - LASTP, LASTP)
        return pltpu.make_async_copy(x_hbm.at[last, rows], xbuf.at[last, rows], rsem.at[last if part == 0 else 0])

    def wr_one(i, r, j, sem):
        col = j * WC if isinstance(j, int) else pl.multiple_of(j * WC, WC)
        return pltpu.make_async_copy(obuf_1.at[pl.ds(slab(i) * nb, nb), pl.ds(r * 8, 8), pl.ds(col, WC)],
                                     out_1.at[pl.ds(i * nb, nb), pl.ds(r * 8, 8), pl.ds(col, WC)], sem)

    def wr_pair(p, r, j):
        ps = p if isinstance(p, int) else jnp.where(p >= NOUT // 2, p - NOUT // 2, p)
        return pltpu.make_async_copy(obuf_2.at[pl.ds(ps * nb, nb), pl.ds(r * 8, 8), pl.ds(j * WC, WC)],
                                     out_2.at[pl.ds(p * nb, nb), pl.ds(r * 8, 8), pl.ds(j * WC, WC)], wsem.at[p])

    def wr_wait(i, n, sem):
        pltpu.make_async_copy(obuf_1.at[pl.ds(slab(i) * nb, n * nb)], out_1.at[pl.ds(i * nb, n * nb)], sem).wait()

    wcp = pltpu.make_async_copy(w_hbm, wbuf, msem.at[0])
    bcp = pltpu.make_async_copy(b_hbm, bbuf, msem.at[1])
    wcp.start()
    bcp.start()
    _loop(0, npc, lambda u: rd_head(u).start())
    _loop(1, last, lambda i: rd(i).start())
    _loop(0, 1, lambda _: rd_last(0).start())
    _loop(0, 1, lambda _: rd_last(1).start())

    wcp.wait()
    bcp.wait()
    _prepare(wbuf, bbuf, a1_ref, a2_ref, bias_ref)

    def small_step(u, tail):
        _once_if(jnp.logical_not(tail), lambda: rd_head(u).wait())
        _once_if(both(tail, u == 0), lambda: rd_last(1).wait())
        for r in range(8):
            for j in range(nj):
                @pl.when(both(tail, u == 0))
                def _():
                    wr_one(last - 1, r, j, wsem.at[npair]).start()
        for r in range(8):
            @pl.when(both(tail, u > 0))
            def _():
                wr_one(last, r, jnp.maximum(u - 1, 0), wsem.at[npair + 1]).start()
        col = pl.multiple_of(u * pw, pw)
        xr = xbuf.at[jnp.where(tail, last, 0), :, pl.ds(col, pw)]
        orf = obuf.at[jnp.where(tail, slab(last), 0), :, pl.ds(col, pw)]
        for k in range(NSMALL):
            _quad(xr, orf, a1_ref, a2_ref, bias_ref, fence_ref, k * QW)

    def big_step(i):
        rd(i).wait()
        _once_if(both(i >= NOUT, band(i, 1) == 0), lambda: wr_wait(i - NOUT, 2, wsem.at[shr(i - NOUT, 1)]))

        def start_writes():
            rd_last(0).wait()
            for u in range(NKICK):
                wr_pair(0, u // nj, u % nj).start()
        _once_if(i == T0, start_writes)

        p = jnp.maximum(i - T0, 0)
        rows = 16 // NPTS
        for k in range(nq):
            if k % (nq // NPTS) == 0:
                r0 = k // (nq // NPTS) * rows
                for r in range(r0, r0 + rows):
                    for j in range(nj):
                        @pl.when(i > T0 if r * nj + j < NKICK else i >= T0)
                        def _():
                            wr_pair(p, r, j).start()
            _quad(xbuf.at[i], obuf.at[slab(i)], a1_ref, a2_ref, bias_ref, fence_ref, k * QW)

    nbig = nbatch - 2

    def step(t):
        tail = t >= npc + nbig
        jax.lax.cond(either(t < npc, tail),
                     lambda: small_step(jnp.where(tail, t - npc - nbig, t), tail),
                     lambda: big_step(t - npc + 1))

    _loop(0, 2 * npc + nbig, step)

    for r in range(8):
        wr_one(last, r, nj - 1, wsem.at[npair + 1]).start()
    for p in range(npair):
        if p not in waited:
            wr_wait(2 * p, 2, wsem.at[p])
    wr_wait(last - 1, 1, wsem.at[npair])
    wr_wait(last, 1, wsem.at[npair + 1])


@jax.jit
def pallas_standalone__structured_sparse_n_m__ragged_kernel(x: jax.Array, w: jax.Array, b: jax.Array):
    nbatch, seq, d = x.shape
    assert d == D and w.shape == (D, D) and b.shape == (D,)
    xt = jnp.transpose(x, (0, 2, 1))
    out_t = pl.pallas_call(
        _kernel,
        in_specs=[pl.BlockSpec(memory_space=pl.ANY)] * 3,
        out_specs=pl.BlockSpec(memory_space=pl.ANY),
        out_shape=jax.ShapeDtypeStruct((nbatch * D // 64, 64, seq), x.dtype),
        scratch_shapes=[
            pltpu.VMEM((nbatch, D, seq), BF16),
            pltpu.VMEM((NOUT, D, seq), BF16),
            pltpu.VMEM((D, D), BF16),
            pltpu.VMEM((D,), BF16),
            pltpu.VMEM((H // 2, 384), U32),
            pltpu.VMEM((Q // 2, 7 * 128 * len(LEVEL2)), U32),
            pltpu.VMEM((D, 128), F32),
            pltpu.SMEM((1,), I32),
            pltpu.SemaphoreType.DMA((nbatch,)),
            pltpu.SemaphoreType.DMA((nbatch // 2 + 1,)),
            pltpu.SemaphoreType.DMA((seq // (NSMALL * QW),)),
            pltpu.SemaphoreType.DMA((2,)),
        ],
        compiler_params=pltpu.CompilerParams(
            vmem_limit_bytes=127 * 1024 * 1024,
            disable_bounds_checks=True,
            disable_semaphore_checks=True,
        ),
    )(xt, w, b)
    return jnp.transpose(out_t.reshape(nbatch, D, seq), (0, 2, 1))
```

```python
import functools

import jax
import jax.numpy as jnp
import jax.experimental.pallas as pl
import jax.experimental.pallas.tpu as pltpu

F32, BF16, U32, I32 = jnp.float32, jnp.bfloat16, jnp.uint32, jnp.int32

D = 576
H = D // 2
Q = H // 2
W1 = 256
W2 = 128
QW = 2 * W1

KW = dict(a=256, b=128, c=256, d=256, e=256, f=256, g22=256, g11=256, g21=128, g12=128)
USES = dict(a=((11, 1), (22, -1)), b=((12, -1), (21, 1)), c=((21, 1), (22, 1)), d=((12, 1), (22, 1)),
            e=((11, 1), (21, 1)), f=((11, 1), (12, 1)), g11=((11, 1),), g22=((22, 1),), g12=((12, 1),),
            g21=((21, 1),))
LEVEL2 = ('a', 'c', 'd', 'e', 'f', 'g22', 'g11')
SWAPPED = ('a', 'd', 'e')
ORDER = ('a', 'b', 'e', 'g21', 'g11', 'f', 'c', 'g12', 'g22', 'd')
A1_OFF = dict(b=0, g21=128, g12=256)
A2_OFF = {g: 7 * 128 * i for i, g in enumerate(LEVEL2)}

NOUT = 10
T0 = 8
LASTP = 48
WC = 1024
NSMALL = 2
NPTS = 4
NKICK = 4


def _swap_pairs(v):
    n, lanes = v.shape
    v3 = v.reshape(n // 8, 8, lanes)
    up = pltpu.roll(v3, 7, 1)
    dn = pltpu.roll(v3, 1, 1)
    odd = (jax.lax.broadcasted_iota(I32, v3.shape, 1) & 1) == 1
    return jnp.where(odd, dn, up).reshape(n, lanes)


def _prune(wb):
    u = pltpu.bitcast(wb, U32)
    lo = pltpu.bitcast((u << 16) & jnp.uint32(0x7FFF0000), F32)
    hi = pltpu.bitcast(u & jnp.uint32(0x7FFF0000), F32)
    big, small = jnp.maximum(lo, hi), jnp.minimum(lo, hi)
    thr = jnp.maximum(jnp.minimum(big, _swap_pairs(big)), jnp.maximum(small, _swap_pairs(small)))
    keep = (jnp.where(lo >= thr, jnp.uint32(0x0000FFFF), jnp.uint32(0))
            | jnp.where(hi >= thr, jnp.uint32(0xFFFF0000), jnp.uint32(0)))
    return pltpu.bitcast(u & keep, BF16)


def _prepare(w_ref, b_ref, a1_ref, a2_ref, bias_ref):
    wp = _prune(w_ref[...])
    r = jnp.concatenate([wp[0:192], wp[384:448], wp[192:384], wp[448:512], wp[512:576], wp[512:576]], axis=0)
    p = r.T.astype(F32)
    a11, a21 = p[:H, 0:256], p[H:, 0:256]
    a12, a22 = p[:H, 256:512], p[H:, 256:512]
    e1, e2 = p[:H, 512:640], p[H:, 512:640]
    low = jax.lax.broadcasted_iota(I32, (H, 128), 1) < 64
    mix = lambda u, v: jnp.concatenate([u[:, :128], jnp.where(low, u[:, 128:], v[:, -128:])], axis=1)
    zero = jnp.zeros((H, 128), F32)
    s1, s6, s7 = a11 + a22, a21 - a11, a12 - a22
    sa = dict(a=mix(s1, zero), b=jnp.where(low, zero, s1[:, 128:]), c=a21 + a22, d=mix(a11, a22), e=mix(a22, a11),
              f=a11 + a12, g22=mix(s6, e2), g11=mix(s7, e1), g21=jnp.where(low, e2, s6[:, 128:]),
              g12=jnp.where(low, e1, s7[:, 128:]))
    for g, m in sa.items():
        if g in LEVEL2:
            p11, p12, p21, p22 = m[:Q, :128], m[:Q, 128:], m[Q:, :128], m[Q:, 128:]
            m = jnp.concatenate([p11 + p22, p21 + p22, p11, p22, p11 + p12, p21 - p11, p12 - p22], axis=1)
            a2_ref[:, A2_OFF[g]:A2_OFF[g] + 7 * 128] = pltpu.bitcast(m.astype(BF16), U32)
        else:
            a1_ref[:, A1_OFF[g]:A1_OFF[g] + KW[g]] = pltpu.bitcast(m.astype(BF16), U32)
    bias_ref[...] = jnp.broadcast_to(b_ref[...].astype(F32).reshape(1, D), (128, D)).T


def _signed_sum(items):
    acc = None
    for sign, get in sorted(items, key=lambda t: -t[0]):
        v = get()
        acc = (v if sign > 0 else -v) if acc is None else (acc + v if sign > 0 else acc - v)
    return acc


def _quad(x_ref, o_ref, a1_ref, a2_ref, bias_ref, fence_ref, c1):
    c2 = c1 + W1
    dot = functools.partial(jnp.dot, preferred_element_type=F32)

    x11, x12, x21, x22 = (0, c1), (0, c2), (192, c1), (192, c2)
    y11, y12, y21, y22 = (384, c1), (384, c2), (448, c1), (448, c2)
    e1, e2 = (512, c1), (512, c2)
    pos, neg = (lambda u: (1,) + u), (lambda u: (-1,) + u)
    operand = dict(
        a=[(192, [pos(x11), neg(x22)]), (64, [])],
        b=[(64, []), (64, [pos(y21), neg(y12)])],
        c=[(192, [pos(x11)]), (64, [pos(y12)])],
        d=[(192, [pos(x12), neg(x22)]), (64, [pos(y22), neg(y12)])],
        e=[(192, [pos(x21), neg(x11)]), (64, [pos(y11), neg(y21)])],
        f=[(192, [pos(x22)]), (64, [pos(y21)])],
        g22=[(192, [pos(x12), neg(x11)]), (64, [pos(e2)])],
        g11=[(192, [pos(x21), neg(x22)]), (64, [pos(e1)])],
        g21=[(64, [pos(e1)]), (64, [pos(y11), neg(y12)])],
        g12=[(64, [pos(e2)]), (64, [pos(y22), neg(y21)])],
    )

    def terms_at(op, row):
        base = 0
        for n, terms in op:
            if base <= row < base + n:
                return [(sg, rr + row - base, cc) for sg, rr, cc in terms]
            base += n

    def tile(op, combo, k, width):
        parts = []
        for lo in range(0, k, 64):
            parts.append([(sg, terms_at(op, r0 + lo), col) for sg, r0, col in combo if terms_at(op, r0 + lo)])
        while not parts[-1]:
            parts.pop()
        load = lambda rr, cc: x_ref[rr:rr + 64, cc:cc + width]
        raw = all(not p or (len(p) == 1 and len(p[0][1]) == 1 and p[0][0] * p[0][1][0][0] > 0) for p in parts)
        out = []
        for p in parts:
            if not p:
                out.append(jnp.zeros((64, width), BF16 if raw else F32))
            elif raw:
                out.append(load(p[0][1][0][1], p[0][1][0][2] + p[0][2]))
            else:
                inner = lambda ts, col: _signed_sum(
                    [(sg, lambda rr=rr, cc=cc: load(rr, cc + col).astype(F32)) for sg, rr, cc in ts])
                out.append(_signed_sum([(sg, lambda ts=ts, col=col: inner(ts, col)) for sg, ts, col in p]))
        return (jnp.concatenate(out, axis=0) if len(out) > 1 else out[0]).astype(BF16)

    def product(g, bias):
        fence_ref[0] = jnp.int32(0)
        op = operand[g]
        if g not in LEVEL2:
            a = pltpu.bitcast(a1_ref[:, A1_OFF[g]:A1_OFF[g] + KW[g]], BF16)
            return dot(a, tile(op, [(1, 0, 0)], KW[g], W1))
        u, v = (W2, 0) if g in SWAPPED else (0, W2)
        combos = ([(1, 0, u), (1, 128, v)], [(1, 0, u)], [(1, 0, v), (-1, 128, v)], [(1, 128, u), (-1, 0, u)],
                  [(1, 128, v)], [(1, 0, u), (1, 0, v)], [(1, 128, u), (1, 128, v)])
        m = {}
        for i in (0, 3, 4, 6, 1, 2, 5):
            t = tile(op, combos[i], 128, W2)
            a = pltpu.bitcast(a2_ref[:, A2_OFF[g] + 128 * i:A2_OFF[g] + 128 * (i + 1)], BF16)
            m[i + 1] = dot(a[:, :t.shape[0]], t)
        g11, g12, g21, g22 = m[1] + m[4] - m[5] + m[7], m[5] + m[3], m[4] + m[2], m[1] - m[2] + m[3] + m[6]
        if g in SWAPPED:
            g11, g12, g21, g22 = g12, g11, g22, g21
        if bias is not None:
            g11, g12, g21, g22 = g11 + bias[:Q], g12 + bias[:Q], g21 + bias[Q:], g22 + bias[Q:]
        return jnp.concatenate([jnp.concatenate([g11, g12], axis=1), jnp.concatenate([g21, g22], axis=1)], axis=0)

    corner = {11: (0, c1), 12: (0, c2), 21: (H, c1), 22: (H, c2)}
    left = {k: 4 for k in corner}
    acc, flipped = {}, {}
    for g in ORDER:
        bias = bias_ref[:H] if g == 'f' else bias_ref[H:] if g == 'c' else None
        v = product(g, bias)
        for k, sign in USES[g]:
            if k not in acc:
                acc[k], flipped[k] = v, sign < 0
            elif flipped[k]:
                assert sign > 0
                acc[k], flipped[k] = v - acc[k], False
            else:
                acc[k] = acc[k] + v if sign > 0 else acc[k] - v
            left[k] -= 1
            if left[k] == 0:
                r0, cc = corner[k]
                o_ref[r0:r0 + H, cc:cc + W1] = acc[k].astype(BF16)


def _loop(lo, hi, f):
    def body(i, carry):
        f(i)
        return carry
    jax.lax.fori_loop(lo, hi, body, 0)


def _once_if(cond, f):
    _loop(0, cond.astype(I32), lambda _: f())


def _kernel(x_hbm, w_hbm, b_hbm, o_hbm, xbuf, obuf, wbuf, bbuf, a1_ref, a2_ref, bias_ref, fence_ref,
            rsem, wsem, hsem, msem):
    nbatch, _, seq = x_hbm.shape
    last = nbatch - 1
    nb = D // 64
    nq, nj = seq // QW, seq // WC
    npc, pw = nq // NSMALL, NSMALL * QW
    npair = (nbatch - 2) // 2
    obuf_1, obuf_2 = obuf.reshape(NOUT * nb, 64, seq), obuf.reshape(NOUT * nb // 2, 128, seq)
    out_1, out_2 = o_hbm, o_hbm.reshape(nbatch * nb // 2, 128, seq)
    band, shr = jax.lax.bitwise_and, jax.lax.shift_right_logical
    both, either = jnp.logical_and, jnp.logical_or

    assert pw == WC and NOUT % 2 == 0 and nbatch <= 2 * NOUT
    assert T0 + npair == last and all(2 * p + 1 < T0 + p for p in range(npair))
    assert all(T0 + (i - NOUT) // 2 < i - i % 2 for i in range(NOUT, nbatch))
    waited = {(i - NOUT) // 2 for i in range(NOUT, last) if i % 2 == 0}
    assert (last - NOUT) // 2 in waited

    def slab(i):
        return i % NOUT if isinstance(i, int) else jnp.where(i >= NOUT, i - NOUT, i)

    def rd_head(u):
        col = pl.multiple_of(u * pw, pw)
        return pltpu.make_async_copy(x_hbm.at[0, :, pl.ds(col, pw)], xbuf.at[0, :, pl.ds(col, pw)], hsem.at[u])

    def rd(i):
        return pltpu.make_async_copy(x_hbm.at[i], xbuf.at[i], rsem.at[i])

    def rd_last(part):
        rows = pl.ds(0, D - LASTP) if part == 0 else pl.ds(D - LASTP, LASTP)
        return pltpu.make_async_copy(x_hbm.at[last, rows], xbuf.at[last, rows], rsem.at[last if part == 0 else 0])

    def wr_one(i, r, j, sem):
        col = j * WC if isinstance(j, int) else pl.multiple_of(j * WC, WC)
        return pltpu.make_async_copy(obuf_1.at[pl.ds(slab(i) * nb, nb), pl.ds(r * 8, 8), pl.ds(col, WC)],
                                     out_1.at[pl.ds(i * nb, nb), pl.ds(r * 8, 8), pl.ds(col, WC)], sem)

    def wr_pair(p, r, j):
        ps = p if isinstance(p, int) else jnp.where(p >= NOUT // 2, p - NOUT // 2, p)
        return pltpu.make_async_copy(obuf_2.at[pl.ds(ps * nb, nb), pl.ds(r * 8, 8), pl.ds(j * WC, WC)],
                                     out_2.at[pl.ds(p * nb, nb), pl.ds(r * 8, 8), pl.ds(j * WC, WC)], wsem.at[p])

    def wr_wait(i, n, sem):
        pltpu.make_async_copy(obuf_1.at[pl.ds(slab(i) * nb, n * nb)], out_1.at[pl.ds(i * nb, n * nb)], sem).wait()

    wcp = pltpu.make_async_copy(w_hbm, wbuf, msem.at[0])
    bcp = pltpu.make_async_copy(b_hbm, bbuf, msem.at[1])
    wcp.start()
    bcp.start()
    _loop(0, npc, lambda u: rd_head(u).start())
    _loop(1, last, lambda i: rd(i).start())
    _loop(0, 1, lambda _: rd_last(0).start())
    _loop(0, 1, lambda _: rd_last(1).start())

    wcp.wait()
    bcp.wait()
    _prepare(wbuf, bbuf, a1_ref, a2_ref, bias_ref)

    def small_step(u, tail):
        _once_if(jnp.logical_not(tail), lambda: rd_head(u).wait())
        _once_if(both(tail, u == 0), lambda: rd_last(1).wait())
        for r in range(8):
            for j in range(nj):
                @pl.when(both(tail, u == 0))
                def _():
                    wr_one(last - 1, r, j, wsem.at[npair]).start()
        for r in range(8):
            @pl.when(both(tail, u > 0))
            def _():
                wr_one(last, r, jnp.maximum(u - 1, 0), wsem.at[npair + 1]).start()
        col = pl.multiple_of(u * pw, pw)
        xr = xbuf.at[jnp.where(tail, last, 0), :, pl.ds(col, pw)]
        orf = obuf.at[jnp.where(tail, slab(last), 0), :, pl.ds(col, pw)]
        for k in range(NSMALL):
            _quad(xr, orf, a1_ref, a2_ref, bias_ref, fence_ref, k * QW)

    def big_step(i):
        rd(i).wait()
        _once_if(both(i >= NOUT, band(i, 1) == 0), lambda: wr_wait(i - NOUT, 2, wsem.at[shr(i - NOUT, 1)]))

        def start_writes():
            rd_last(0).wait()
            for u in range(NKICK):
                wr_pair(0, u // nj, u % nj).start()
        _once_if(i == T0, start_writes)

        p = jnp.maximum(i - T0, 0)
        rows = 16 // NPTS
        for k in range(nq):
            if k % (nq // NPTS) == 0:
                r0 = k // (nq // NPTS) * rows
                for r in range(r0, r0 + rows):
                    for j in range(nj):
                        @pl.when(i > T0 if r * nj + j < NKICK else i >= T0)
                        def _():
                            wr_pair(p, r, j).start()
            _quad(xbuf.at[i], obuf.at[slab(i)], a1_ref, a2_ref, bias_ref, fence_ref, k * QW)

    nbig = nbatch - 2

    def step(t):
        tail = t >= npc + nbig
        jax.lax.cond(either(t < npc, tail),
                     lambda: small_step(jnp.where(tail, t - npc - nbig, t), tail),
                     lambda: big_step(t - npc + 1))

    _loop(0, 2 * npc + nbig, step)

    for r in range(8):
        wr_one(last, r, nj - 1, wsem.at[npair + 1]).start()
    for p in range(npair):
        if p not in waited:
            wr_wait(2 * p, 2, wsem.at[p])
    wr_wait(last - 1, 1, wsem.at[npair])
    wr_wait(last, 1, wsem.at[npair + 1])


@jax.jit
def pallas_standalone__structured_sparse_n_m__ragged_kernel(x: jax.Array, w: jax.Array, b: jax.Array):
    nbatch, seq, d = x.shape
    assert d == D and w.shape == (D, D) and b.shape == (D,)
    xt = jnp.transpose(x, (0, 2, 1))
    out_t = pl.pallas_call(
        _kernel,
        in_specs=[pl.BlockSpec(memory_space=pl.ANY)] * 3,
        out_specs=pl.BlockSpec(memory_space=pl.ANY),
        out_shape=jax.ShapeDtypeStruct((nbatch * D // 64, 64, seq), x.dtype),
        scratch_shapes=[
            pltpu.VMEM((nbatch, D, seq), BF16),
            pltpu.VMEM((NOUT, D, seq), BF16),
            pltpu.VMEM((D, D), BF16),
            pltpu.VMEM((D,), BF16),
            pltpu.VMEM((H // 2, 384), U32),
            pltpu.VMEM((Q // 2, 7 * 128 * len(LEVEL2)), U32),
            pltpu.VMEM((D, 128), F32),
            pltpu.SMEM((1,), I32),
            pltpu.SemaphoreType.DMA((nbatch,)),
            pltpu.SemaphoreType.DMA((nbatch // 2 + 1,)),
            pltpu.SemaphoreType.DMA((seq // (NSMALL * QW),)),
            pltpu.SemaphoreType.DMA((2,)),
        ],
        compiler_params=pltpu.CompilerParams(
            vmem_limit_bytes=127 * 1024 * 1024,
            disable_bounds_checks=True,
            disable_semaphore_checks=True,
        ),
    )(xt, w, b)
    return jnp.transpose(out_t.reshape(nbatch, D, seq), (0, 2, 1))
```

```python
import functools

import jax
import jax.numpy as jnp
import jax.experimental.pallas as pl
import jax.experimental.pallas.tpu as pltpu

F32, BF16, U32, I32 = jnp.float32, jnp.bfloat16, jnp.uint32, jnp.int32

D = 576
H = D // 2
Q = H // 2
W1 = 256
W2 = 128
QW = 2 * W1

KW = dict(a=256, b=128, c=256, d=256, e=256, f=256, g22=256, g11=256, g21=128, g12=128)
USES = dict(a=((11, 1), (22, -1)), b=((12, -1), (21, 1)), c=((21, 1), (22, 1)), d=((12, 1), (22, 1)),
            e=((11, 1), (21, 1)), f=((11, 1), (12, 1)), g11=((11, 1),), g22=((22, 1),), g12=((12, 1),),
            g21=((21, 1),))
LEVEL2 = ('a', 'c', 'd', 'e', 'f', 'g22', 'g11')
SWAPPED = ('a', 'd', 'e')
ORDER = ('a', 'b', 'e', 'g21', 'g11', 'f', 'c', 'g12', 'g22', 'd')
A1_OFF = dict(b=0, g21=128, g12=256)
A2_OFF = {g: 7 * 128 * i for i, g in enumerate(LEVEL2)}

NOUT = 10
T0 = 8
LASTP = 48
WC = 1024
NSMALL = 2
NPTS = 4
NKICK = 4


def _swap_pairs(v):
    n, lanes = v.shape
    v3 = v.reshape(n // 8, 8, lanes)
    up = pltpu.roll(v3, 7, 1)
    dn = pltpu.roll(v3, 1, 1)
    odd = (jax.lax.broadcasted_iota(I32, v3.shape, 1) & 1) == 1
    return jnp.where(odd, dn, up).reshape(n, lanes)


def _prune(wb):
    u = pltpu.bitcast(wb, U32)
    lo = pltpu.bitcast((u << 16) & jnp.uint32(0x7FFF0000), F32)
    hi = pltpu.bitcast(u & jnp.uint32(0x7FFF0000), F32)
    big, small = jnp.maximum(lo, hi), jnp.minimum(lo, hi)
    thr = jnp.maximum(jnp.minimum(big, _swap_pairs(big)), jnp.maximum(small, _swap_pairs(small)))
    keep = (jnp.where(lo >= thr, jnp.uint32(0x0000FFFF), jnp.uint32(0))
            | jnp.where(hi >= thr, jnp.uint32(0xFFFF0000), jnp.uint32(0)))
    return pltpu.bitcast(u & keep, BF16)


def _prepare(w_ref, b_ref, a1_ref, a2_ref, bias_ref):
    wp = _prune(w_ref[...])
    r = jnp.concatenate([wp[0:192], wp[384:448], wp[192:384], wp[448:512], wp[512:576], wp[512:576]], axis=0)
    p = r.T.astype(F32)
    a11, a21 = p[:H, 0:256], p[H:, 0:256]
    a12, a22 = p[:H, 256:512], p[H:, 256:512]
    e1, e2 = p[:H, 512:640], p[H:, 512:640]
    low = jax.lax.broadcasted_iota(I32, (H, 128), 1) < 64
    mix = lambda u, v: jnp.concatenate([u[:, :128], jnp.where(low, u[:, 128:], v[:, -128:])], axis=1)
    zero = jnp.zeros((H, 128), F32)
    s1, s6, s7 = a11 + a22, a21 - a11, a12 - a22
    sa = dict(a=mix(s1, zero), b=jnp.where(low, zero, s1[:, 128:]), c=a21 + a22, d=mix(a11, a22), e=mix(a22, a11),
              f=a11 + a12, g22=mix(s6, e2), g11=mix(s7, e1), g21=jnp.where(low, e2, s6[:, 128:]),
              g12=jnp.where(low, e1, s7[:, 128:]))
    for g, m in sa.items():
        if g in LEVEL2:
            p11, p12, p21, p22 = m[:Q, :128], m[:Q, 128:], m[Q:, :128], m[Q:, 128:]
            m = jnp.concatenate([p11 + p22, p21 + p22, p11, p22, p11 + p12, p21 - p11, p12 - p22], axis=1)
            a2_ref[:, A2_OFF[g]:A2_OFF[g] + 7 * 128] = pltpu.bitcast(m.astype(BF16), U32)
        else:
            a1_ref[:, A1_OFF[g]:A1_OFF[g] + KW[g]] = pltpu.bitcast(m.astype(BF16), U32)
    bias_ref[...] = jnp.broadcast_to(b_ref[...].astype(F32).reshape(1, D), (128, D)).T


def _signed_sum(items):
    acc = None
    for sign, get in sorted(items, key=lambda t: -t[0]):
        v = get()
        acc = (v if sign > 0 else -v) if acc is None else (acc + v if sign > 0 else acc - v)
    return acc


def _quad(x_ref, o_ref, a1_ref, a2_ref, bias_ref, fence_ref, c1):
    c2 = c1 + W1
    dot = functools.partial(jnp.dot, preferred_element_type=F32)

    x11, x12, x21, x22 = (0, c1), (0, c2), (192, c1), (192, c2)
    y11, y12, y21, y22 = (384, c1), (384, c2), (448, c1), (448, c2)
    e1, e2 = (512, c1), (512, c2)
    pos, neg = (lambda u: (1,) + u), (lambda u: (-1,) + u)
    operand = dict(
        a=[(192, [pos(x11), neg(x22)]), (64, [])],
        b=[(64, []), (64, [pos(y21), neg(y12)])],
        c=[(192, [pos(x11)]), (64, [pos(y12)])],
        d=[(192, [pos(x12), neg(x22)]), (64, [pos(y22), neg(y12)])],
        e=[(192, [pos(x21), neg(x11)]), (64, [pos(y11), neg(y21)])],
        f=[(192, [pos(x22)]), (64, [pos(y21)])],
        g22=[(192, [pos(x12), neg(x11)]), (64, [pos(e2)])],
        g11=[(192, [pos(x21), neg(x22)]), (64, [pos(e1)])],
        g21=[(64, [pos(e1)]), (64, [pos(y11), neg(y12)])],
        g12=[(64, [pos(e2)]), (64, [pos(y22), neg(y21)])],
    )

    def terms_at(op, row):
        base = 0
        for n, terms in op:
            if base <= row < base + n:
                return [(sg, rr + row - base, cc) for sg, rr, cc in terms]
            base += n

    def tile(op, combo, k, width):
        parts = []
        for lo in range(0, k, 64):
            parts.append([(sg, terms_at(op, r0 + lo), col) for sg, r0, col in combo if terms_at(op, r0 + lo)])
        while not parts[-1]:
            parts.pop()
        load = lambda rr, cc: x_ref[rr:rr + 64, cc:cc + width]
        raw = all(not p or (len(p) == 1 and len(p[0][1]) == 1 and p[0][0] * p[0][1][0][0] > 0) for p in parts)
        out = []
        for p in parts:
            if not p:
                out.append(jnp.zeros((64, width), BF16 if raw else F32))
            elif raw:
                out.append(load(p[0][1][0][1], p[0][1][0][2] + p[0][2]))
            else:
                inner = lambda ts, col: _signed_sum(
                    [(sg, lambda rr=rr, cc=cc: load(rr, cc + col).astype(F32)) for sg, rr, cc in ts])
                out.append(_signed_sum([(sg, lambda ts=ts, col=col: inner(ts, col)) for sg, ts, col in p]))
        return (jnp.concatenate(out, axis=0) if len(out) > 1 else out[0]).astype(BF16)

    def product(g, bias):
        fence_ref[0] = jnp.int32(0)
        op = operand[g]
        if g not in LEVEL2:
            a = pltpu.bitcast(a1_ref[:, A1_OFF[g]:A1_OFF[g] + KW[g]], BF16)
            return dot(a, tile(op, [(1, 0, 0)], KW[g], W1))
        u, v = (W2, 0) if g in SWAPPED else (0, W2)
        combos = ([(1, 0, u), (1, 128, v)], [(1, 0, u)], [(1, 0, v), (-1, 128, v)], [(1, 128, u), (-1, 0, u)],
                  [(1, 128, v)], [(1, 0, u), (1, 0, v)], [(1, 128, u), (1, 128, v)])
        m = {}
        for i in (0, 3, 4, 6, 1, 2, 5):
            t = tile(op, combos[i], 128, W2)
            a = pltpu.bitcast(a2_ref[:, A2_OFF[g] + 128 * i:A2_OFF[g] + 128 * (i + 1)], BF16)
            m[i + 1] = dot(a[:, :t.shape[0]], t)
        g11, g12, g21, g22 = m[1] + m[4] - m[5] + m[7], m[5] + m[3], m[4] + m[2], m[1] - m[2] + m[3] + m[6]
        if g in SWAPPED:
            g11, g12, g21, g22 = g12, g11, g22, g21
        if bias is not None:
            g11, g12, g21, g22 = g11 + bias[:Q], g12 + bias[:Q], g21 + bias[Q:], g22 + bias[Q:]
        return jnp.concatenate([jnp.concatenate([g11, g12], axis=1), jnp.concatenate([g21, g22], axis=1)], axis=0)

    corner = {11: (0, c1), 12: (0, c2), 21: (H, c1), 22: (H, c2)}
    left = {k: 4 for k in corner}
    acc, flipped = {}, {}
    for g in ORDER:
        bias = bias_ref[:H] if g == 'f' else bias_ref[H:] if g == 'c' else None
        v = product(g, bias)
        for k, sign in USES[g]:
            if k not in acc:
                acc[k], flipped[k] = v, sign < 0
            elif flipped[k]:
                assert sign > 0
                acc[k], flipped[k] = v - acc[k], False
            else:
                acc[k] = acc[k] + v if sign > 0 else acc[k] - v
            left[k] -= 1
            if left[k] == 0:
                r0, cc = corner[k]
                o_ref[r0:r0 + H, cc:cc + W1] = acc[k].astype(BF16)


def _loop(lo, hi, f):
    def body(i, carry):
        f(i)
        return carry
    jax.lax.fori_loop(lo, hi, body, 0)


def _once_if(cond, f):
    _loop(0, cond.astype(I32), lambda _: f())


def _kernel(x_hbm, w_hbm, b_hbm, o_hbm, xbuf, obuf, wbuf, bbuf, a1_ref, a2_ref, bias_ref, fence_ref,
            rsem, wsem, hsem, msem):
    nbatch, _, seq = x_hbm.shape
    last = nbatch - 1
    nb = D // 64
    nq, nj = seq // QW, seq // WC
    npc, pw = nq // NSMALL, NSMALL * QW
    npair = (nbatch - 2) // 2
    obuf_1, obuf_2 = obuf.reshape(NOUT * nb, 64, seq), obuf.reshape(NOUT * nb // 2, 128, seq)
    out_1, out_2 = o_hbm, o_hbm.reshape(nbatch * nb // 2, 128, seq)
    band, shr = jax.lax.bitwise_and, jax.lax.shift_right_logical
    both, either = jnp.logical_and, jnp.logical_or

    assert pw == WC and NOUT % 2 == 0 and nbatch <= 2 * NOUT
    assert T0 + npair == last and all(2 * p + 1 < T0 + p for p in range(npair))
    assert all(T0 + (i - NOUT) // 2 < i - i % 2 for i in range(NOUT, nbatch))
    waited = {(i - NOUT) // 2 for i in range(NOUT, last) if i % 2 == 0}
    assert (last - NOUT) // 2 in waited

    def slab(i):
        return i % NOUT if isinstance(i, int) else jnp.where(i >= NOUT, i - NOUT, i)

    def rd_head(u):
        col = pl.multiple_of(u * pw, pw)
        return pltpu.make_async_copy(x_hbm.at[0, :, pl.ds(col, pw)], xbuf.at[0, :, pl.ds(col, pw)], hsem.at[u])

    def rd(i):
        return pltpu.make_async_copy(x_hbm.at[i], xbuf.at[i], rsem.at[i])

    def rd_last(part):
        rows = pl.ds(0, D - LASTP) if part == 0 else pl.ds(D - LASTP, LASTP)
        return pltpu.make_async_copy(x_hbm.at[last, rows], xbuf.at[last, rows], rsem.at[last if part == 0 else 0])

    def wr_one(i, r, j, sem):
        col = j * WC if isinstance(j, int) else pl.multiple_of(j * WC, WC)
        return pltpu.make_async_copy(obuf_1.at[pl.ds(slab(i) * nb, nb), pl.ds(r * 8, 8), pl.ds(col, WC)],
                                     out_1.at[pl.ds(i * nb, nb), pl.ds(r * 8, 8), pl.ds(col, WC)], sem)

    def wr_pair(p, r, j):
        ps = p if isinstance(p, int) else jnp.where(p >= NOUT // 2, p - NOUT // 2, p)
        return pltpu.make_async_copy(obuf_2.at[pl.ds(ps * nb, nb), pl.ds(r * 8, 8), pl.ds(j * WC, WC)],
                                     out_2.at[pl.ds(p * nb, nb), pl.ds(r * 8, 8), pl.ds(j * WC, WC)], wsem.at[p])

    def wr_wait(i, n, sem):
        pltpu.make_async_copy(obuf_1.at[pl.ds(slab(i) * nb, n * nb)], out_1.at[pl.ds(i * nb, n * nb)], sem).wait()

    wcp = pltpu.make_async_copy(w_hbm, wbuf, msem.at[0])
    bcp = pltpu.make_async_copy(b_hbm, bbuf, msem.at[1])
    wcp.start()
    bcp.start()
    _loop(0, npc, lambda u: rd_head(u).start())
    _loop(1, last, lambda i: rd(i).start())
    _loop(0, 1, lambda _: rd_last(0).start())
    _loop(0, 1, lambda _: rd_last(1).start())

    wcp.wait()
    bcp.wait()
    _prepare(wbuf, bbuf, a1_ref, a2_ref, bias_ref)

    def small_step(u, tail):
        _once_if(jnp.logical_not(tail), lambda: rd_head(u).wait())
        _once_if(both(tail, u == 0), lambda: rd_last(1).wait())
        for r in range(8):
            for j in range(nj):
                @pl.when(both(tail, u == 0))
                def _():
                    wr_one(last - 1, r, j, wsem.at[npair]).start()
        for r in range(8):
            @pl.when(both(tail, u > 0))
            def _():
                wr_one(last, r, jnp.maximum(u - 1, 0), wsem.at[npair + 1]).start()
        col = pl.multiple_of(u * pw, pw)
        xr = xbuf.at[jnp.where(tail, last, 0), :, pl.ds(col, pw)]
        orf = obuf.at[jnp.where(tail, slab(last), 0), :, pl.ds(col, pw)]
        for k in range(NSMALL):
            _quad(xr, orf, a1_ref, a2_ref, bias_ref, fence_ref, k * QW)

    def big_step(i):
        rd(i).wait()
        _once_if(both(i >= NOUT, band(i, 1) == 0), lambda: wr_wait(i - NOUT, 2, wsem.at[shr(i - NOUT, 1)]))

        def start_writes():
            rd_last(0).wait()
            for u in range(NKICK):
                wr_pair(0, u // nj, u % nj).start()
        _once_if(i == T0, start_writes)

        p = jnp.maximum(i - T0, 0)
        rows = 16 // NPTS
        for k in range(nq):
            if k % (nq // NPTS) == 0:
                r0 = k // (nq // NPTS) * rows
                for r in range(r0, r0 + rows):
                    for j in range(nj):
                        @pl.when(i > T0 if r * nj + j < NKICK else i >= T0)
                        def _():
                            wr_pair(p, r, j).start()
            _quad(xbuf.at[i], obuf.at[slab(i)], a1_ref, a2_ref, bias_ref, fence_ref, k * QW)

    nbig = nbatch - 2

    def step(t):
        tail = t >= npc + nbig
        jax.lax.cond(either(t < npc, tail),
                     lambda: small_step(jnp.where(tail, t - npc - nbig, t), tail),
                     lambda: big_step(t - npc + 1))

    _loop(0, 2 * npc + nbig, step)

    for r in range(8):
        wr_one(last, r, nj - 1, wsem.at[npair + 1]).start()
    for p in range(npair):
        if p not in waited:
            wr_wait(2 * p, 2, wsem.at[p])
    wr_wait(last - 1, 1, wsem.at[npair])
    wr_wait(last, 1, wsem.at[npair + 1])


def _compiler_params():
    base = dict(vmem_limit_bytes=127 * 1024 * 1024, disable_bounds_checks=True)
    try:
        return pltpu.CompilerParams(disable_semaphore_checks=True, **base)
    except TypeError:
        return pltpu.CompilerParams(**base)


@jax.jit
def pallas_standalone__structured_sparse_n_m__ragged_kernel(x: jax.Array, w: jax.Array, b: jax.Array):
    nbatch, seq, d = x.shape
    assert d == D and w.shape == (D, D) and b.shape == (D,)
    xt = jnp.transpose(x, (0, 2, 1))
    out_t = pl.pallas_call(
        _kernel,
        in_specs=[pl.BlockSpec(memory_space=pl.ANY)] * 3,
        out_specs=pl.BlockSpec(memory_space=pl.ANY),
        out_shape=jax.ShapeDtypeStruct((nbatch * D // 64, 64, seq), x.dtype),
        scratch_shapes=[
            pltpu.VMEM((nbatch, D, seq), BF16),
            pltpu.VMEM((NOUT, D, seq), BF16),
            pltpu.VMEM((D, D), BF16),
            pltpu.VMEM((D,), BF16),
            pltpu.VMEM((H // 2, 384), U32),
            pltpu.VMEM((Q // 2, 7 * 128 * len(LEVEL2)), U32),
            pltpu.VMEM((D, 128), F32),
            pltpu.SMEM((1,), I32),
            pltpu.SemaphoreType.DMA((nbatch,)),
            pltpu.SemaphoreType.DMA((nbatch // 2 + 1,)),
            pltpu.SemaphoreType.DMA((seq // (NSMALL * QW),)),
            pltpu.SemaphoreType.DMA((2,)),
        ],
        compiler_params=_compiler_params(),
    )(xt, w, b)
    return jnp.transpose(out_t.reshape(nbatch, D, seq), (0, 2, 1))
```
